```python
import os as _os
_os.environ.setdefault("JAX_PLATFORMS", "cpu")
import jax
import jax.numpy as jnp

def _softmax(x, axis=-1):
    return jax.nn.softmax(x, axis=axis)
def _gelu(x):
    return jax.nn.gelu(x, approximate=True)
def _silu(x):
    return jax.nn.silu(x)
def _sigmoid(x):
    return jax.nn.sigmoid(x)
def _layernorm(x, axis=-1, eps=1e-5):
    m = jnp.mean(x, axis=axis, keepdims=True)
    v = jnp.var(x, axis=axis, keepdims=True)
    return (x - m) / jnp.sqrt(v + eps)
def _scatter_add(tgt, idx, src, axis=0):
    return tgt.at[idx].add(src)
def _segment_sum(src, seg, n):
    return jax.ops.segment_sum(src, seg, n)
class _Rng:
    def __init__(self, key):
        self._k = key
    def _next(self):
        self._k, sub = jax.random.split(self._k)
        return sub
    def normal(self, shape):
        return jax.random.normal(self._next(), shape, dtype=jnp.bfloat16)
    def randint(self, lo, hi, shape):
        return jax.random.randint(self._next(), shape, lo, hi, dtype=jnp.int32)
    def uniform(self, shape, lo=0.0, hi=1.0):
        return jax.random.uniform(self._next(), shape, jnp.bfloat16, lo, hi)
    def permutation(self, n):
        return jax.random.permutation(self._next(), n)


kernel_name = 'concat_heads__compressed_kv_cla__compressed_kv_cla__decode'

def setup_inputs():
    _rng = _Rng(jax.random.key(int.from_bytes(__import__("os").urandom(4), "little")))
    _w = (lambda a: (lambda t: t.astype(jnp.bfloat16) if jnp.issubdtype(t.dtype, jnp.floating) else t)(jnp.asarray(a)))
    def _A_setup():
        B, H, Sq, Sk, D, M = 4, 32, 1, 4096, 128, 640
        Dc = 4 * D
        return {
            "x": _w((lambda *s: _rng.normal(s) * 1.6)(B, Sq, M)),
            "c_kv": _w((lambda *s: _rng.normal(s) * 0.05)(B, Sk, Dc)),
            "w_q": _w((lambda *s: _rng.normal(s) * 1.6)(M, H, D) * (M ** -0.5)),
            "w_uk": _w((lambda *s: _rng.normal(s) * 1.6)(Dc, H, D) * (Dc ** -0.5)),
            "w_uv": _w((lambda *s: _rng.normal(s) * 0.05)(Dc, H, D) * (Dc ** -0.5)),
            "w_o": _w((lambda *s: _rng.normal(s) * 0.05)(H, D, M) * ((H * D) ** -0.5)),
        }
    _A_in = _A_setup()

    def _B_setup():
        B, H, Sq, Sk, D, M = 4, 32, 1, 4096, 128, 640
        Dc = 4 * D
        return {
            "x": _w((lambda *s: _rng.normal(s) * 1.6)(B, Sq, M)),
            "c_kv": _w((lambda *s: _rng.normal(s) * 0.05)(B, Sk, Dc)),
            "w_q": _w((lambda *s: _rng.normal(s) * 1.6)(M, H, D) * (M ** -0.5)),
            "w_uk": _w((lambda *s: _rng.normal(s) * 1.6)(Dc, H, D) * (Dc ** -0.5)),
            "w_uv": _w((lambda *s: _rng.normal(s) * 0.05)(Dc, H, D) * (Dc ** -0.5)),
            "w_o": _w((lambda *s: _rng.normal(s) * 0.05)(H, D, M) * ((H * D) ** -0.5)),
        }
    _B_in = _B_setup()

    return {
        "A_x": _A_in["x"],
        "A_c_kv": _A_in["c_kv"],
        "A_w_q": _A_in["w_q"],
        "A_w_uk": _A_in["w_uk"],
        "A_w_uv": _A_in["w_uv"],
        "A_w_o": _A_in["w_o"],
        "B_x": _B_in["x"],
        "B_c_kv": _B_in["c_kv"],
        "B_w_q": _B_in["w_q"],
        "B_w_uk": _B_in["w_uk"],
        "B_w_uv": _B_in["w_uv"],
        "B_w_o": _B_in["w_o"],
    }

def reference(A_x, A_c_kv, A_w_q, A_w_uk, A_w_uv, A_w_o, B_x, B_c_kv, B_w_q, B_w_uk, B_w_uv, B_w_o):
    def _A_ref(x, c_kv, w_q, w_uk, w_uv, w_o):
        B, Sq, M = x.shape[0], x.shape[1], x.shape[2]
        Sk = c_kv.shape[1]
        H, D = w_q.shape[1], w_q.shape[2]
        q = jnp.einsum("bqm,mhd->bhqd", x, w_q)
        k = jnp.einsum("bkc,chd->bhkd", c_kv, w_uk)
        v = jnp.einsum("bkc,chd->bhkd", c_kv, w_uv)
        scores = jnp.einsum("bhqd,bhkd->bhqk", q, k) * (D ** -0.5)
        off = Sk - Sq
        qi = jnp.arange(Sq)[:, None]
        kj = jnp.arange(Sk)[None, :]
        cmask = kj <= (qi + off)
        scores = jnp.where(cmask[None, None], scores, -1e9)
        p = _softmax(scores, axis=-1)
        ctx = jnp.einsum("bhqk,bhkd->bhqd", p, v)
        return jnp.einsum("bhqd,hdm->bqm", ctx, w_o)

    def _B_ref(x, c_kv, w_q, w_uk, w_uv, w_o):
        B, Sq, M = x.shape[0], x.shape[1], x.shape[2]
        Sk = c_kv.shape[1]
        H, D = w_q.shape[1], w_q.shape[2]
        q = jnp.einsum("bqm,mhd->bhqd", x, w_q)
        k = jnp.einsum("bkc,chd->bhkd", c_kv, w_uk)
        v = jnp.einsum("bkc,chd->bhkd", c_kv, w_uv)
        scores = jnp.einsum("bhqd,bhkd->bhqk", q, k) * (D ** -0.5)
        off = Sk - Sq
        qi = jnp.arange(Sq)[:, None]
        kj = jnp.arange(Sk)[None, :]
        cmask = kj <= (qi + off)
        scores = jnp.where(cmask[None, None], scores, -1e9)
        p = _softmax(scores, axis=-1)
        ctx = jnp.einsum("bhqk,bhkd->bhqd", p, v)
        return jnp.einsum("bhqd,hdm->bqm", ctx, w_o)

    a = _A_ref(A_x, A_c_kv, A_w_q, A_w_uk, A_w_uv, A_w_o)
    b = _B_ref(B_x, B_c_kv, B_w_q, B_w_uk, B_w_uv, B_w_o)
    return jnp.concatenate([a, b], axis=-1)
```

```python
import functools
import jax
import jax.numpy as jnp
from jax import lax
import jax.experimental.pallas as pl
import jax.experimental.pallas.tpu as pltpu

f32, bf16 = jnp.float32, jnp.bfloat16
B, H, SK, D, M, DC = 4, 32, 4096, 128, 640, 512
BH = B * H

CFG = dict(CH_Q=4096, CH_K=4096, CH_V=4096, O_PIECES=(3072, 768, 256), O_STEP=256, NOSEMCHK=True, FIRST_OUT=True, CKV_G=2)


def _iota(shape, dim):
    return lax.broadcasted_iota(jnp.int32, shape, dim)


def _dmask(rows):
    return (_iota((rows, BH), 0) & (H - 1)) == (_iota((rows, BH), 1) & (H - 1))


import contextlib
def build(cfg):
    scope = (lambda n: jax.named_scope(n)) if cfg.get('SCOPES') else (lambda n: contextlib.nullcontext())
    CH_Q, CH_K, CH_V = cfg['CH_Q'], cfg['CH_K'], cfg['CH_V']
    O_PIECES, O_STEP = cfg['O_PIECES'], cfg['O_STEP']
    assert sum(O_PIECES) == H * D
    scale = float(D) ** -0.5
    CKV_G = cfg.get('CKV_G', 1)
    NPRIO1 = cfg.get('NPRIO1', 0)
    FIRST_OUT = cfg.get('FIRST_OUT', False)

    def kernel(xa_hbm, ckva_hbm, wqa_hbm, wuka_hbm, wuva_hbm, woa_hbm,
               xb_hbm, ckvb_hbm, wqb_hbm, wukb_hbm, wuvb_hbm, wob_hbm,
               o_ref,
               x_buf, wq_buf, wuk_buf, ckv_buf, wuv_buf, wo_buf,
               xs_ref, g_ref, acc_ref, qat_ref, qabs_ref, ctxc_ref, lo_ref, oacc_ref,
               sem_x, sem_wq, sem_wuk, sem_ckv, sem_wuv, sem_wo):
        xh = (xa_hbm, xb_hbm); ckvh = (ckva_hbm, ckvb_hbm); wqh = (wqa_hbm, wqb_hbm)
        wukh = (wuka_hbm, wukb_hbm); wuvh = (wuva_hbm, wuvb_hbm); woh = (woa_hbm, wob_hbm)

        copies = []
        for br in range(2):
            copies.append((wqh[br], wq_buf.at[br], sem_wq.at[br]))
            if br == 0:
                for i in range(2):
                    copies.append((xh[i], x_buf.at[i], sem_x.at[i]))
            copies.append((wukh[br], wuk_buf.at[br], sem_wuk.at[br]))
            for b in range(0, B, CKV_G):
                copies.append((ckvh[br].at[pl.ds(b, CKV_G)], ckv_buf.at[pl.ds(br * B + b, CKV_G)], sem_ckv.at[(br * B + b) // CKV_G]))
        for br in range(2):
            copies.append((wuvh[br], wuv_buf.at[br], sem_wuv.at[br]))
        copies.append((woh[0], wo_buf.at[0], sem_wo.at[0]))
        off = 0
        for i, n in enumerate(O_PIECES):
            copies.append((woh[1].at[pl.ds(off, n)], wo_buf.at[1, pl.ds(off, n)], sem_wo.at[1 + i]))
            off += n

        k0 = 0
        if FIRST_OUT:
            pltpu.make_async_copy(*copies[0]).start()
            k0 = 1

        def issue(i, _):
            for k, (src, dst, sem) in enumerate(copies):
                if k < k0:
                    continue
                @pl.when(i == k)
                def _():
                    pltpu.make_async_copy(src, dst, sem).start(priority=1 if k >= len(copies) - NPRIO1 else 0)
            return 0
        with scope('issue'):
            lax.fori_loop(k0, len(copies), issue, 0)

        def wait(buf, sem, name='wait'):
            with scope(name):
                pltpu.make_async_copy(buf, buf, sem).wait()

        def expand_matmul(w_buf, br, nrows, ch):
            jper = ch // H
            acc_ref[...] = jnp.zeros_like(acc_ref)

            def body(i, _):
                w = w_buf[br, pl.ds(pl.multiple_of(i * ch, ch), ch), :]
                g = g_ref[pl.ds(pl.multiple_of(i * jper, jper), jper), :]
                lt = jnp.broadcast_to(g[:, None, :], (jper, H, BH)).reshape(ch, BH)
                lt = jnp.where(_dmask(ch), lt, 0.0).astype(bf16)
                acc_ref[...] += lax.dot_general(lt, w, (((0,), (0,)), ((), ())), preferred_element_type=f32)
                return 0
            lax.fori_loop(0, nrows // ch, body, 0)

        xs_ref[...] = jnp.zeros_like(xs_ref)

        def attention(br, _):
            wait(x_buf.at[br], sem_x.at[br], 'w_x')
            xs_ref[0:B, :] = x_buf[br].astype(f32)
            e128 = jnp.where(_iota((BH, BH), 0) == (_iota((BH, BH), 1) >> 5), 1.0, 0.0).astype(bf16)
            g_ref[...] = jnp.dot(xs_ref[...].T.astype(bf16), e128, preferred_element_type=f32)
            wait(wq_buf.at[br], sem_wq.at[br], 'w_wq')
            with scope('Q'):
                expand_matmul(wq_buf, br, M * H, CH_Q)
            q = acc_ref[...].astype(bf16)

            wait(wuk_buf.at[br], sem_wuk.at[br], 'w_wuk')
            cper = CH_K // H

            def kbody(i, _):
                w = wuk_buf[br, pl.ds(pl.multiple_of(i * CH_K, CH_K), CH_K), :]
                r = lax.dot_general(w, q, (((1,), (1,)), ((), ())), preferred_element_type=f32)
                r = jnp.where(_dmask(CH_K), r, 0.0)
                qat_ref[pl.ds(pl.multiple_of(i * cper, cper), cper), :] = jnp.sum(r.reshape(cper, H, BH), axis=1)
                return 0
            with scope('K'):
                lax.fori_loop(0, DC * H // CH_K, kbody, 0)
            qabs_ref[...] = (qat_ref[...] * scale).T.astype(bf16)

            def bbody(b, _):
                idx = br * B + b
                if CKV_G == 1:
                    wait(ckv_buf.at[idx], sem_ckv.at[idx], 'w_ckv')
                else:
                    @pl.when(b % CKV_G == 0)
                    def _():
                        wait(ckv_buf.at[pl.ds(idx, CKV_G)], sem_ckv.at[idx // CKV_G], 'w_ckv')
                c = ckv_buf[idx]
                qb = qabs_ref[pl.ds(pl.multiple_of(b * H, H), H), :]
                s = lax.dot_general(qb, c, (((1,), (1,)), ((), ())), preferred_element_type=f32)
                m = jnp.max(s, axis=1, keepdims=True)
                p = jnp.exp(s - m)
                l = jnp.sum(p, axis=1, keepdims=True)
                cc = jnp.dot(p.astype(bf16), c, preferred_element_type=f32)
                ctxc_ref[br, pl.ds(pl.multiple_of(b * H, H), H), :] = cc / l
                return 0
            lax.fori_loop(0, B, bbody, 0)
            return 0
        lax.fori_loop(0, 2, attention, 0)

        def vstage(br, _):
            g_ref[0:DC, :] = ctxc_ref[br].T
            wait(wuv_buf.at[br], sem_wuv.at[br], 'w_wuv')
            with scope('V'):
                expand_matmul(wuv_buf, br, DC * H, CH_V)
            lo_ref[br] = acc_ref[...].reshape(B, H * D)
            return 0
        lax.fori_loop(0, 2, vstage, 0)

        def obranch(br, _):
            @pl.when(br == 0)
            def _():
                wait(wo_buf.at[0], sem_wo.at[0], 'w_wo')
            acc = None
            off = 0
            for i, n in enumerate(O_PIECES):
                @pl.when(br == 1)
                def _():
                    wait(wo_buf.at[1, pl.ds(off, n)], sem_wo.at[1 + i], 'w_wo1')
                with scope('O1'):
                    lhs = lo_ref[br, :, off:off + n].astype(bf16)
                    part = jnp.dot(lhs, wo_buf[br, off:off + n, :], preferred_element_type=f32)
                    if i == 0:
                        oacc_ref[...] = part
                    elif i < len(O_PIECES) - 1:
                        oacc_ref[...] += part
                    else:
                        res = (oacc_ref[...] + part).astype(o_ref.dtype)
                        @pl.when(br == 0)
                        def _():
                            o_ref[:, 0:M] = res
                        @pl.when(br == 1)
                        def _():
                            o_ref[:, M:2 * M] = res
                off += n
            return 0
        lax.fori_loop(0, 2, obranch, 0)

    @jax.jit
    def fn(A_x, A_c_kv, A_w_q, A_w_uk, A_w_uv, A_w_o, B_x, B_c_kv, B_w_q, B_w_uk, B_w_uv, B_w_o):
        def prep(x, ckv, wq, wuk, wuv, wo):
            return (x.reshape(B, M), ckv, wq.reshape(M * H, D), wuk.reshape(DC * H, D),
                    wuv.reshape(DC * H, D), wo.reshape(H * D, M))
        args = prep(A_x, A_c_kv, A_w_q, A_w_uk, A_w_uv, A_w_o) + prep(B_x, B_c_kv, B_w_q, B_w_uk, B_w_uv, B_w_o)
        out = pl.pallas_call(
            kernel,
            out_shape=jax.ShapeDtypeStruct((B, 2 * M), bf16),
            in_specs=[pl.BlockSpec(memory_space=pl.ANY)] * 12,
            out_specs=pl.BlockSpec(memory_space=pltpu.VMEM),
            scratch_shapes=[
                pltpu.VMEM((2, B, M), bf16),
                pltpu.VMEM((2, M * H, D), bf16),
                pltpu.VMEM((2, DC * H, D), bf16),
                pltpu.VMEM((2 * B, SK, DC), bf16),
                pltpu.VMEM((2, DC * H, D), bf16),
                pltpu.VMEM((2, H * D, M), bf16),
                pltpu.VMEM((BH, M), f32),
                pltpu.VMEM((M, BH), f32),
                pltpu.VMEM((BH, D), f32),
                pltpu.VMEM((DC, BH), f32),
                pltpu.VMEM((BH, DC), bf16),
                pltpu.VMEM((2, BH, DC), f32),
                pltpu.VMEM((2, B, H * D), f32),
                pltpu.VMEM((B, M), f32),
                pltpu.SemaphoreType.DMA((2,)),
                pltpu.SemaphoreType.DMA((2,)),
                pltpu.SemaphoreType.DMA((2,)),
                pltpu.SemaphoreType.DMA((2 * B // CKV_G,)),
                pltpu.SemaphoreType.DMA((2,)),
                pltpu.SemaphoreType.DMA((1 + len(O_PIECES),)),
            ],
            compiler_params=pltpu.CompilerParams(vmem_limit_bytes=100 * 1024 * 1024, disable_semaphore_checks=cfg.get('NOSEMCHK', False), disable_bounds_checks=cfg.get('NOBND', False)),
        )(*args)
        return out.reshape(B, 1, 2 * M)
    return fn


pallas_concat_heads__compressed_kv_cla__compressed_kv_cla__decode_kernel = build(CFG)
```

```python
import jax
import jax.numpy as jnp
from jax import lax
import jax.experimental.pallas as pl
import jax.experimental.pallas.tpu as pltpu

f32, bf16 = jnp.float32, jnp.bfloat16

B, H, SK, D, M, DC = 4, 32, 4096, 128, 640, 512
BH = B * H
CH = 4096
O_PIECES = (3072, 640, 256, 128)
NT = (((1,), (1,)), ((), ()))
TN = (((0,), (0,)), ((), ()))


def _iota(shape, dim):
    return lax.broadcasted_iota(jnp.int32, shape, dim)


def _head_diag(rows):
    return (_iota((rows, BH), 0) & (H - 1)) == (_iota((rows, BH), 1) & (H - 1))


def _kernel(xa_hbm, ckva_hbm, wqa_hbm, wuka_hbm, wuva_hbm, woa_hbm,
            xb_hbm, ckvb_hbm, wqb_hbm, wukb_hbm, wuvb_hbm, wob_hbm,
            o_ref,
            x_buf, wq_buf, wuk_buf, ckv_buf, wuv_buf, wo_buf,
            xs_ref, g_ref, acc_ref, qat_ref, qabs_ref, cc_ref, ctx_ref, oacc_ref,
            sem_x, sem_wq, sem_wuk, sem_ckv, sem_wuv, sem_wo):
    x_hbm, ckv_hbm, wq_hbm = (xa_hbm, xb_hbm), (ckva_hbm, ckvb_hbm), (wqa_hbm, wqb_hbm)
    wuk_hbm, wuv_hbm, wo_hbm = (wuka_hbm, wukb_hbm), (wuva_hbm, wuvb_hbm), (woa_hbm, wob_hbm)

    copies = []
    for br in range(2):
        copies.append((wq_hbm[br], wq_buf.at[br], sem_wq.at[br]))
        if br == 0:
            copies += [(x_hbm[i], x_buf.at[i], sem_x.at[i]) for i in range(2)]
        copies.append((wuk_hbm[br], wuk_buf.at[br], sem_wuk.at[br]))
        copies += [(ckv_hbm[br].at[b], ckv_buf.at[br * B + b], sem_ckv.at[br * B + b]) for b in range(B)]
    copies += [(wuv_hbm[br], wuv_buf.at[br], sem_wuv.at[br]) for br in range(2)]
    copies.append((wo_hbm[0], wo_buf.at[0], sem_wo.at[0]))
    off = 0
    for i, n in enumerate(O_PIECES):
        copies.append((wo_hbm[1].at[pl.ds(off, n)], wo_buf.at[1, pl.ds(off, n)], sem_wo.at[1 + i]))
        off += n

    pltpu.make_async_copy(*copies[0]).start()

    def issue(i, carry):
        for k in range(1, len(copies)):
            @pl.when(i == k)
            def _():
                pltpu.make_async_copy(*copies[k]).start()
        return carry
    lax.fori_loop(1, len(copies), issue, 0)

    def wait(dst, sem):
        pltpu.make_async_copy(dst, dst, sem).wait()

    def headwise_matmul(w_buf, br, nrows):
        jper = CH // H
        acc_ref[...] = jnp.zeros_like(acc_ref)

        def body(i, carry):
            w = w_buf[br, pl.ds(pl.multiple_of(i * CH, CH), CH), :]
            g = g_ref[pl.ds(pl.multiple_of(i * jper, jper), jper), :]
            lt = jnp.broadcast_to(g[:, None, :], (jper, H, BH)).reshape(CH, BH)
            lt = jnp.where(_head_diag(CH), lt, 0.0).astype(bf16)
            acc_ref[...] += lax.dot_general(lt, w, TN, preferred_element_type=f32)
            return carry
        lax.fori_loop(0, nrows // CH, body, 0)

    xs_ref[...] = jnp.zeros_like(xs_ref)

    def attention(br, carry):
        wait(x_buf.at[br], sem_x.at[br])
        xs_ref[0:B, :] = x_buf[br].astype(f32)
        spread = jnp.where(_iota((BH, BH), 0) == (_iota((BH, BH), 1) >> 5), 1.0, 0.0).astype(bf16)
        g_ref[...] = jnp.dot(xs_ref[...].T.astype(bf16), spread, preferred_element_type=f32)
        wait(wq_buf.at[br], sem_wq.at[br])
        headwise_matmul(wq_buf, br, M * H)
        q = acc_ref[...].astype(bf16)

        wait(wuk_buf.at[br], sem_wuk.at[br])
        cper = CH // H

        def absorb(i, c2):
            w = wuk_buf[br, pl.ds(pl.multiple_of(i * CH, CH), CH), :]
            r = lax.dot_general(w, q, NT, preferred_element_type=f32)
            r = jnp.where(_head_diag(CH), r, 0.0)
            qat_ref[pl.ds(pl.multiple_of(i * cper, cper), cper), :] = jnp.sum(r.reshape(cper, H, BH), axis=1)
            return c2
        lax.fori_loop(0, DC * H // CH, absorb, 0)
        qabs_ref[...] = (qat_ref[...] * (float(D) ** -0.5)).T.astype(bf16)

        def attend(b, c2):
            idx = br * B + b
            rows = pl.ds(pl.multiple_of(b * H, H), H)
            wait(ckv_buf.at[idx], sem_ckv.at[idx])
            c = ckv_buf[idx]
            s = lax.dot_general(qabs_ref[rows, :], c, NT, preferred_element_type=f32)
            p = jnp.exp(s - jnp.max(s, axis=1, keepdims=True))
            l = jnp.sum(p, axis=1, keepdims=True)
            cc_ref[br, rows, :] = jnp.dot(p.astype(bf16), c, preferred_element_type=f32) / l
            return c2
        lax.fori_loop(0, B, attend, 0)
        return carry
    lax.fori_loop(0, 2, attention, 0)

    def value_up(br, carry):
        g_ref[0:DC, :] = cc_ref[br].T
        wait(wuv_buf.at[br], sem_wuv.at[br])
        headwise_matmul(wuv_buf, br, DC * H)
        ctx_ref[br] = acc_ref[...].reshape(B, H * D)
        return carry
    lax.fori_loop(0, 2, value_up, 0)

    wait(wo_buf.at[0], sem_wo.at[0])
    o_ref[:, 0:M] = jnp.dot(ctx_ref[0].astype(bf16), wo_buf[0], preferred_element_type=f32).astype(o_ref.dtype)
    off = 0
    for i, n in enumerate(O_PIECES):
        lhs = ctx_ref[1, :, off:off + n].astype(bf16)
        prev = oacc_ref[...] if i > 0 else None
        wait(wo_buf.at[1, pl.ds(off, n)], sem_wo.at[1 + i])
        part = jnp.dot(lhs, wo_buf[1, off:off + n, :], preferred_element_type=f32)
        if i > 0:
            part = prev + part
        if i < len(O_PIECES) - 1:
            oacc_ref[...] = part
        else:
            o_ref[:, M:2 * M] = part.astype(o_ref.dtype)
        off += n


def _compiler_params():
    vmem = 100 * 1024 * 1024
    try:
        return pltpu.CompilerParams(vmem_limit_bytes=vmem, disable_semaphore_checks=True)
    except TypeError:
        return pltpu.CompilerParams(vmem_limit_bytes=vmem)


@jax.jit
def pallas_concat_heads__compressed_kv_cla__compressed_kv_cla__decode_kernel(
    A_x: jax.Array,
    A_c_kv: jax.Array,
    A_w_q: jax.Array,
    A_w_uk: jax.Array,
    A_w_uv: jax.Array,
    A_w_o: jax.Array,
    B_x: jax.Array,
    B_c_kv: jax.Array,
    B_w_q: jax.Array,
    B_w_uk: jax.Array,
    B_w_uv: jax.Array,
    B_w_o: jax.Array,
):
    def views(x, ckv, wq, wuk, wuv, wo):
        return (x.reshape(B, M), ckv, wq.reshape(M * H, D), wuk.reshape(DC * H, D),
                wuv.reshape(DC * H, D), wo.reshape(H * D, M))

    args = (views(A_x, A_c_kv, A_w_q, A_w_uk, A_w_uv, A_w_o)
            + views(B_x, B_c_kv, B_w_q, B_w_uk, B_w_uv, B_w_o))
    dma_sems = pltpu.SemaphoreType.DMA
    out = pl.pallas_call(
        _kernel,
        out_shape=jax.ShapeDtypeStruct((B, 2 * M), bf16),
        in_specs=[pl.BlockSpec(memory_space=pl.ANY)] * 12,
        out_specs=pl.BlockSpec(memory_space=pltpu.VMEM),
        scratch_shapes=[
            pltpu.VMEM((2, B, M), bf16),
            pltpu.VMEM((2, M * H, D), bf16),
            pltpu.VMEM((2, DC * H, D), bf16),
            pltpu.VMEM((2 * B, SK, DC), bf16),
            pltpu.VMEM((2, DC * H, D), bf16),
            pltpu.VMEM((2, H * D, M), bf16),
            pltpu.VMEM((BH, M), f32),
            pltpu.VMEM((M, BH), f32),
            pltpu.VMEM((BH, D), f32),
            pltpu.VMEM((DC, BH), f32),
            pltpu.VMEM((BH, DC), bf16),
            pltpu.VMEM((2, BH, DC), f32),
            pltpu.VMEM((2, B, H * D), f32),
            pltpu.VMEM((B, M), f32),
            dma_sems((2,)), dma_sems((2,)), dma_sems((2,)), dma_sems((2 * B,)), dma_sems((2,)),
            dma_sems((1 + len(O_PIECES),)),
        ],
        compiler_params=_compiler_params(),
    )(*args)
    return out.reshape(B, 1, 2 * M)
```
